```python
import jax
import jax.numpy as jnp

def _softmax(x, axis=-1):
    return jax.nn.softmax(x, axis=axis)

def _gelu(x):
    return jax.nn.gelu(x, approximate=True)

def _silu(x):
    return jax.nn.silu(x)

def _sigmoid(x):
    return jax.nn.sigmoid(x)

def _layernorm(x, axis=-1, eps=1e-05):
    m = jnp.mean(x, axis=axis, keepdims=True)
    v = jnp.var(x, axis=axis, keepdims=True)
    return (x - m) / jnp.sqrt(v + eps)

def _scatter_add(tgt, idx, src, axis=0):
    return tgt.at[idx].add(src)

def _segment_sum(src, seg, n):
    return jax.ops.segment_sum(src, seg, n)

class _Rng:

    def __init__(self, key):
        self._k = key

    def _next(self):
        self._k, sub = jax.random.split(self._k)
        return sub

    def normal(self, shape):
        return jax.random.normal(self._next(), shape, dtype=jnp.bfloat16)

    def randint(self, lo, hi, shape):
        return jax.random.randint(self._next(), shape, lo, hi, dtype=jnp.int32)

    def uniform(self, shape, lo=0.0, hi=1.0):
        return jax.random.uniform(self._next(), shape, jnp.bfloat16, lo, hi)

    def permutation(self, n):
        return jax.random.permutation(self._next(), n)
kernel_name = 'adaLN_cond__mha_block_cached__moe_arch_mod__decode'

def setup_inputs():
    _rng = _Rng(jax.random.key(int.from_bytes(__import__("os").urandom(4), "little")))
    _w = lambda a: (lambda t: t.astype(jnp.bfloat16) if jnp.issubdtype(t.dtype, jnp.floating) else t)(jnp.asarray(a))

    def _A_setup():
        B, Sq, D = (4, 1, 448)
        H, Sk, Dh = (16, 16384, 256)
        return {'x': _w((lambda *s: _rng.normal(s) * 0.05)(B, Sq, D)), 'k_cache': _w((lambda *s: _rng.normal(s) * 0.05)(B, H, Sk, Dh)), 'v_cache': _w((lambda *s: _rng.normal(s) * 0.05)(B, H, Sk, Dh)), 'wq': _w((lambda *s: _rng.normal(s) * 0.05)(D, H * Dh) * D ** (-0.5)), 'wo': _w((lambda *s: _rng.normal(s) * 0.05)(H * Dh, D) * (H * Dh) ** (-0.5))}
    _A_in = _A_setup()

    def _B_setup():
        B, S, D, F, C = (4, 1, 448, 1792, 1)
        return {'x': _w((lambda *s: _rng.normal(s) * 0.05)(B, S, D)), 'w_r': _w((lambda *s: _rng.normal(s) * 0.05)(D)), 'w_gate': _w((lambda *s: _rng.normal(s) * 0.05)(D, F)), 'w_up': _w((lambda *s: _rng.normal(s) * 0.05)(D, F)), 'w_down': _w((lambda *s: _rng.normal(s) * 0.05)(F, D))}
    _B_in = _B_setup()
    return {'A_x': _A_in['x'], 'A_k_cache': _A_in['k_cache'], 'A_v_cache': _A_in['v_cache'], 'A_wq': _A_in['wq'], 'A_wo': _A_in['wo'], 'B_x': _B_in['x'], 'B_w_r': _B_in['w_r'], 'B_w_gate': _B_in['w_gate'], 'B_w_up': _B_in['w_up'], 'B_w_down': _B_in['w_down'], 'c': _w((lambda *s: _rng.normal(s) * 0.05)(4, 448)), 'w_mod': _w((lambda *s: _rng.normal(s) * 0.05)(448, 6 * 448) * 448 ** (-0.5))}

def reference(A_x, A_k_cache, A_v_cache, A_wq, A_wo, B_x, B_w_r, B_w_gate, B_w_up, B_w_down, c, w_mod):

    def _A_ref(x, k_cache, v_cache, wq, wo):
        B, Sq, D = x.shape
        H, Dh = (16, 256)
        q = (lambda x, *d: x.transpose(*d))((x @ wq).reshape(B, Sq, H, Dh), 0, 2, 1, 3)
        scores = jnp.einsum('bhqd,bhkd->bhqk', q, k_cache) * Dh ** (-0.5)
        p = _softmax(scores, axis=-1)
        o = jnp.einsum('bhqk,bhkd->bhqd', p, v_cache)
        return (lambda x, *d: x.transpose(*d))(o, 0, 2, 1, 3).reshape(B, Sq, H * Dh) @ wo

    def _B_ref(x, w_r, w_gate, w_up, w_down):
        B, S, D = x.shape
        C = 1
        r = x @ w_r
        idx = jnp.argsort(-r, axis=-1)[:, :C]
        idx_e = jnp.repeat(idx.reshape(B, C, 1), D, axis=2)
        x_sel = jnp.take_along_axis(x, idx_e, axis=1)
        g = _silu(x_sel @ w_gate)
        u = x_sel @ w_up
        y = g * u @ w_down
        r_sel = _sigmoid(jnp.take_along_axis(r, idx, axis=1))
        y = y * r_sel.reshape(B, C, 1)
        b_off = (jnp.arange(B) * S).reshape(B, 1)
        flat_idx = (idx + b_off).reshape(B * C)
        zero = (x * 0.0).reshape(B * S, D)
        upd = _scatter_add(zero, flat_idx, y.reshape(B * C, D), axis=0)
        return x + upd.reshape(B, S, D)
    x = A_x
    mod = (_silu(c) @ w_mod).reshape(c.shape[0], 6, 1, -1)
    sa, ca, ga, sb, cb, gb = (mod[:, 0].copy(), mod[:, 1].copy(), mod[:, 2].copy(), mod[:, 3].copy(), mod[:, 4].copy(), mod[:, 5].copy())
    h = _layernorm(x, axis=-1) * (1 + ca) + sa
    x = x + ga * _A_ref(h, A_k_cache, A_v_cache, A_wq, A_wo)
    h = _layernorm(x, axis=-1) * (1 + cb) + sb
    x = x + gb * _B_ref(h, B_w_r, B_w_gate, B_w_up, B_w_down)
    return x
```

```python
import jax
import jax.numpy as jnp
import jax.experimental.pallas as pl
import jax.experimental.pallas.tpu as pltpu

f32, bf16 = jnp.float32, jnp.bfloat16


def _ln(x):
    m = jnp.mean(x, axis=-1, keepdims=True)
    xc = x - m
    v = jnp.mean(xc * xc, axis=-1, keepdims=True)
    return xc / jnp.sqrt(v + 1e-5)


def _dot(a, b):
    return jnp.dot(a, b, preferred_element_type=f32)


def _dot_t(a, b):
    return jax.lax.dot_general(a, b, (((1,), (1,)), ((), ())), preferred_element_type=f32)


def _make(PR=128, P=32, splits=((96, 128, 1), (0, 96, 0)), G=4):
    B, D, H, SK, DH = 4, 448, 16, 16384, 256
    BLK = PR * P
    BPH = SK // BLK
    NBLK = B * H * BPH

    def kernel(x_ref, c_ref, wr_ref, k_hbm, v_hbm, wmod_hbm, wq_hbm, wo_hbm, wg_hbm, wu_hbm, wd_hbm,
               out_ref,
               kbuf, vbuf, wmod_b, wq_b, wo_b, wg_b, wu_b, wd_b, q_scr, o_scr, ksem, vsem, wsem):

        def issue(src, buf, sem, g, p):
            base = pl.multiple_of(g * BLK, BLK) + p * PR
            for a, b, pr in splits:
                pltpu.make_async_copy(src.at[pl.ds(base + a, b - a)], buf.at[p, pl.ds(a, b - a)],
                                      sem.at[p]).start(priority=pr)

        def wait(src, buf, sem, p):
            pltpu.make_async_copy(src.at[pl.ds(0, PR)], buf.at[p], sem.at[p]).wait()

        wcopies = [pltpu.make_async_copy(s, d, wsem.at[i]) for i, (s, d) in enumerate(
            [(wmod_hbm, wmod_b), (wq_hbm, wq_b), (wo_hbm, wo_b), (wg_hbm, wg_b), (wu_hbm, wu_b), (wd_hbm, wd_b)])]
        wcopies[0].start(priority=0)
        wcopies[1].start(priority=1)
        for p in range(P):
            issue(k_hbm, kbuf, ksem, 0, p)
            issue(v_hbm, vbuf, vsem, 0, p)
        for i, w in enumerate(wcopies[2:]):
            w.start(priority=i % 2)

        x = x_ref[...].astype(f32)
        c = c_ref[...].astype(f32)
        sc = c * jax.nn.sigmoid(c)
        wcopies[0].wait()
        mod = _dot(sc.astype(bf16), wmod_b[...])
        sa, ca, ga, sb, cb, gb = [mod[:, i * D:(i + 1) * D] for i in range(6)]
        h = _ln(x) * (1 + ca) + sa
        wcopies[1].wait()
        q = _dot(h.astype(bf16), wq_b[...]).astype(bf16).astype(f32) * (DH ** -0.5)
        q_scr[...] = jnp.zeros(q_scr.shape, f32)
        o_scr[...] = jnp.zeros(o_scr.shape, f32)
        for hh in range(H):
            q_scr[hh, 0:B, :] = q[:, hh * DH:(hh + 1) * DH]

        row = jax.lax.broadcasted_iota(jnp.int32, (8, DH), 0)

        def step(g, carry, do_k, k_issue, do_v, v_issue, k_prev, v_prev):
            m, l, acc, pc = carry
            ss, pv = [], []
            if do_k:
                qh = q_scr[((g + 1) // BPH) % H].astype(bf16)
            for p0 in range(0, P, G):
                for p in range(p0, p0 + G):
                    pp = (p - G) % P
                    gk = g + 1 if p0 > 0 else g
                    ki = (k_issue if p0 > 0 else k_prev)
                    vi = (v_issue if p0 > 0 else v_prev)
                    if do_k:
                        wait(k_hbm, kbuf, ksem, p)
                    if ki:
                        issue(k_hbm, kbuf, ksem, gk + 1, pp)
                    if do_v:
                        wait(v_hbm, vbuf, vsem, p)
                    if vi:
                        issue(v_hbm, vbuf, vsem, gk, pp)
                rows = slice(p0 * PR, (p0 + G) * PR)
                if do_k:
                    ss.append(_dot_t(qh, kbuf[p0:p0 + G].reshape(G * PR, DH)))
                if do_v:
                    acc = acc + _dot(pc[:, rows], vbuf[p0:p0 + G].reshape(G * PR, DH))
            if do_v:
                bh = g // BPH
                hh = bh % H
                o_scr[hh] = jnp.where(row == bh // H, acc / l, o_scr[hh])
            if do_k:
                first = (g + 1) % BPH == 0
                s = jnp.concatenate(ss, axis=1)
                m_old = jnp.where(first, -jnp.inf, m)
                m = jnp.maximum(m_old, jnp.max(s, axis=-1, keepdims=True))
                alpha = jnp.exp(m_old - m)
                pe = jnp.exp(s - m)
                pc = pe.astype(bf16)
                l = jnp.where(first, 0.0, l * alpha) + jnp.sum(pe, axis=-1, keepdims=True)
                acc = jnp.where(first, 0.0, acc * alpha)
            return m, l, acc, pc

        carry = (jnp.full((8, 1), -jnp.inf, f32), jnp.zeros((8, 1), f32), jnp.zeros((8, DH), f32),
                 jnp.zeros((8, BLK), bf16))
        T, N = True, False
        carry = step(-1, carry, T, T, N, N, N, N)
        carry = step(0, carry, T, T, T, T, T, N)
        carry = jax.lax.fori_loop(1, NBLK - 2, lambda g, cr: step(g, cr, T, T, T, T, T, T), carry)
        carry = step(NBLK - 2, carry, T, N, T, T, T, T)
        step(NBLK - 1, carry, N, N, T, N, N, T)

        for w in wcopies[2:]:
            w.wait()
        o = jnp.concatenate([o_scr[hh][0:B] for hh in range(H)], axis=1)
        a = _dot_t(o.astype(bf16), wo_b[...])
        x1 = x + ga * a
        h2 = _ln(x1) * (1 + cb) + sb
        h2b = h2.astype(bf16)
        r = jnp.sum(h2 * wr_ref[...].astype(f32).reshape(1, D), axis=-1, keepdims=True)
        gate = _dot(h2b, wg_b[...])
        gate = gate * jax.nn.sigmoid(gate)
        u = _dot(h2b, wu_b[...])
        y = _dot_t((gate * u).astype(bf16), wd_b[...])
        y = y * jax.nn.sigmoid(r)
        out_ref[...] = (x1 + gb * (h2 + y)).astype(out_ref.dtype)

    @jax.jit
    def pallas_adaLN_cond__mha_block_cached__moe_arch_mod__decode_kernel(
            A_x, A_k_cache, A_v_cache, A_wq, A_wo, B_x, B_w_r, B_w_gate, B_w_up, B_w_down, c, w_mod):
        hbm = pl.BlockSpec(memory_space=pltpu.HBM)
        vm = pl.BlockSpec(memory_space=pltpu.VMEM)
        wo_t, wd_t = A_wo.T, B_w_down.T
        out = pl.pallas_call(
            kernel,
            out_shape=jax.ShapeDtypeStruct((B, D), A_x.dtype),
            in_specs=[vm, vm, vm] + [hbm] * 8,
            out_specs=vm,
            scratch_shapes=[
                pltpu.VMEM((P, PR, DH), bf16), pltpu.VMEM((P, PR, DH), bf16),
                pltpu.VMEM(w_mod.shape, bf16), pltpu.VMEM(A_wq.shape, bf16), pltpu.VMEM(wo_t.shape, bf16),
                pltpu.VMEM(B_w_gate.shape, bf16), pltpu.VMEM(B_w_up.shape, bf16), pltpu.VMEM(wd_t.shape, bf16),
                pltpu.VMEM((H, 8, DH), f32), pltpu.VMEM((H, 8, DH), f32),
                pltpu.SemaphoreType.DMA((P,)), pltpu.SemaphoreType.DMA((P,)), pltpu.SemaphoreType.DMA((6,)),
            ],
            compiler_params=pltpu.CompilerParams(vmem_limit_bytes=64 * 1024 * 1024),
        )(A_x.reshape(B, D), c, B_w_r, A_k_cache.reshape(B * H * SK, DH), A_v_cache.reshape(B * H * SK, DH),
          w_mod, A_wq, wo_t, B_w_gate, B_w_up, wd_t)
        return out.reshape(B, 1, D)

    return pallas_adaLN_cond__mha_block_cached__moe_arch_mod__decode_kernel


pallas_adaLN_cond__mha_block_cached__moe_arch_mod__decode_kernel = _make()
```
